```python
import jax
import jax.numpy as jnp

def _softmax(x, axis=-1):
    return jax.nn.softmax(x, axis=axis)
def _gelu(x):
    return jax.nn.gelu(x, approximate=True)
def _silu(x):
    return jax.nn.silu(x)
def _sigmoid(x):
    return jax.nn.sigmoid(x)
def _layernorm(x, axis=-1, eps=1e-5):
    m = jnp.mean(x, axis=axis, keepdims=True)
    v = jnp.var(x, axis=axis, keepdims=True)
    return (x - m) / jnp.sqrt(v + eps)
def _scatter_add(tgt, idx, src, axis=0):
    return tgt.at[idx].add(src)
def _segment_sum(src, seg, n):
    return jax.ops.segment_sum(src, seg, n)
class _Rng:
    def __init__(self, key):
        self._k = key
    def _next(self):
        self._k, sub = jax.random.split(self._k)
        return sub
    def normal(self, shape):
        return jax.random.normal(self._next(), shape, dtype=jnp.bfloat16)
    def randint(self, lo, hi, shape):
        return jax.random.randint(self._next(), shape, lo, hi, dtype=jnp.int32)
    def uniform(self, shape, lo=0.0, hi=1.0):
        return jax.random.uniform(self._next(), shape, jnp.bfloat16, lo, hi)
    def permutation(self, n):
        return jax.random.permutation(self._next(), n)


kernel_name = 'standalone__depthwise_separable__vision'

def setup_inputs():
    _rng = _Rng(jax.random.key(int.from_bytes(__import__("os").urandom(4), "little")))
    _w = (lambda a: (lambda t: t.astype(jnp.bfloat16) if jnp.issubdtype(t.dtype, jnp.floating) else t)(jnp.asarray(a)))
    H = W = 384
    C = 384
    k = 1
    return {
        "x": _w((lambda *s: _rng.normal(s) * 0.05)(1, H, W, C)),
        "dw": _w((lambda *s: _rng.normal(s) * 0.05)(k, k, C)),
        "pw": _w((lambda *s: _rng.normal(s) * 0.05)(C, C)),
    }

def reference(x, dw, pw):
    B, H, W, C = x.shape
    k = dw.shape[0]
    pad = k // 2
    xp = jnp.pad(x, ((0,0),(pad,pad),(pad,pad),(0,0)))
    out = jnp.zeros_like(x)
    for i in range(k):
        for j in range(k):
            out = out + xp[:, i:i+H, j:j+W, :] * dw[i, j][None, None, None, :]
    return jnp.einsum('bhwc,cd->bhwd', out, pw)
```

```python
import jax
import jax.numpy as jnp
from jax import lax
import jax.experimental.pallas as pl
import jax.experimental.pallas.tpu as pltpu

_GROUPS = 36
_WRITE_ROWS = 32
_STEP_ROWS = 64
_AHEAD = 2
_FIRST_WRITES = 4


@jax.jit
def pallas_standalone__depthwise_separable__vision_kernel(
    x: jax.Array,
    dw: jax.Array,
    pw: jax.Array,
):
    B, H, W, C = x.shape
    assert dw.shape == (1, 1, C) and pw.shape == (C, C)
    G, wseg, cseg = _GROUPS, _WRITE_ROWS, _STEP_ROWS
    R = B * H * W // G
    assert G * R == B * H * W and R % (2 * cseg) == 0
    n_steps = R // cseg
    n_writes = R // wseg
    per_step = cseg // wseg
    half = n_steps // 2

    def kernel(x_hbm, dw_hbm, pw_hbm, o_hbm, buf, dw_v, pw_v,
               rsem, bsem, wsem, psem):
        def read(i):
            s = pl.ds(pl.multiple_of(i * cseg, cseg), cseg)
            return pltpu.make_async_copy(
                x_hbm.at[:, s], buf.at[:, s], rsem.at[i % (_AHEAD + 1)])

        def write(i):
            s = pl.ds(pl.multiple_of(i * wseg, wseg), wseg)
            return pltpu.make_async_copy(buf.at[:, s], o_hbm.at[:, s], wsem)

        def compute(i):
            s = pl.ds(pl.multiple_of(i * cseg, cseg), cseg)
            t = buf[:, s, :].reshape(G * cseg, C) * dw_v[0]
            y = jnp.dot(t, pw_v[...], preferred_element_type=jnp.float32)
            buf[:, s, :] = y.astype(buf.dtype).reshape(G, cseg, C)

        second = pl.ds(half * cseg, R - half * cseg)
        background = pltpu.make_async_copy(
            x_hbm.at[:, second], buf.at[:, second], bsem)
        dw_copy = pltpu.make_async_copy(dw_hbm, dw_v, psem.at[0])
        pw_copy = pltpu.make_async_copy(pw_hbm, pw_v, psem.at[1])

        background.start(priority=1)
        for i in range(_AHEAD):
            read(i).start()
        dw_copy.start()
        pw_copy.start()
        dw_copy.wait()
        pw_copy.wait()

        def read_phase(i, _):
            @pl.when(i + _AHEAD < half)
            def _():
                read(i + _AHEAD).start()
            read(i).wait()
            compute(i)

        lax.fori_loop(0, half, read_phase, None)
        background.wait()

        for k in range(_FIRST_WRITES):
            write(k).start()

        def write_phase(i, _):
            compute(i)
            base = _FIRST_WRITES + (i - half) * 2 * per_step
            for k in range(2 * per_step):
                @pl.when(base + k < n_writes - per_step)
                def _():
                    write(base + k).start()

        lax.fori_loop(half, n_steps, write_phase, None)
        for k in range(n_writes - per_step, n_writes):
            write(k).start()
        pltpu.make_async_copy(buf, o_hbm, wsem).wait()

    hbm = pl.BlockSpec(memory_space=pltpu.HBM)
    out = pl.pallas_call(
        kernel,
        in_specs=[hbm, hbm, hbm],
        out_specs=hbm,
        out_shape=jax.ShapeDtypeStruct((G, R, C), x.dtype),
        scratch_shapes=[
            pltpu.VMEM((G, R, C), x.dtype),
            pltpu.VMEM(dw.shape, dw.dtype),
            pltpu.VMEM(pw.shape, pw.dtype),
            pltpu.SemaphoreType.DMA((_AHEAD + 1,)),
            pltpu.SemaphoreType.DMA,
            pltpu.SemaphoreType.DMA,
            pltpu.SemaphoreType.DMA((2,)),
        ],
        compiler_params=pltpu.CompilerParams(vmem_limit_bytes=120 << 20),
    )(x.reshape(G, R, C), dw, pw)
    return out.reshape(B, H, W, C)
```

```python
import functools

import jax
import jax.numpy as jnp
from jax import lax
import jax.experimental.pallas as pl
import jax.experimental.pallas.tpu as pltpu

_GROUPS = 6
_CHUNK_ROWS = 384
_READ_ROWS = 32
_WRITE_ROWS = 48
_PREFETCH = 8


def _read_batches(n_chunks, read_steps):
    edges = [0, 2]
    while edges[-1] < read_steps:
        edges.append(min(2 * edges[-1], n_chunks - 1))
    if edges[-1] < n_chunks - 1:
        edges.append(n_chunks - 1)
    edges.append(n_chunks)
    for lo, hi in zip(edges, edges[1:]):
        assert lo >= read_steps or hi <= _PREFETCH + 2 * lo
    return edges


@jax.jit
def pallas_standalone__depthwise_separable__vision_kernel(
    x: jax.Array,
    dw: jax.Array,
    pw: jax.Array,
):
    B, H, W, C = x.shape
    assert dw.shape == (1, 1, C) and pw.shape == (C, C)
    rows = B * H * W // _GROUPS
    n_chunks = rows // _CHUNK_ROWS
    assert _GROUPS * n_chunks * _CHUNK_ROWS == B * H * W
    assert (n_chunks - _PREFETCH) % 2 == 0
    read_steps = (n_chunks - _PREFETCH) // 2
    edges = _read_batches(n_chunks, read_steps)
    n_batches = len(edges) - 1

    def kernel(x_hbm, dw_hbm, pw_hbm, o_hbm,
               buf, dw_vmem, pw_vmem, read_sems, write_sem, weight_sems):
        def row_slice(chunk, part, size):
            start = chunk * _CHUNK_ROWS + part * size
            return pl.ds(pl.multiple_of(start, size), size)

        def start_read(chunk):
            batch = sum(jnp.where(chunk >= e, 1, 0) for e in edges[1:-1])
            for part in range(_CHUNK_ROWS // _READ_ROWS):
                r = row_slice(chunk, part, _READ_ROWS)
                for queue in range(2):
                    g = pl.ds(queue * (_GROUPS // 2), _GROUPS // 2)
                    pltpu.make_async_copy(
                        x_hbm.at[g, r], buf.at[g, r], read_sems.at[batch]
                    ).start(priority=queue)

        def wait_batch(batch):
            lo, hi = edges[batch], edges[batch + 1]
            r = pl.ds(lo * _CHUNK_ROWS, (hi - lo) * _CHUNK_ROWS)
            pltpu.make_async_copy(
                x_hbm.at[:, r], buf.at[:, r], read_sems.at[batch]
            ).wait()

        def start_write(chunk):
            for part in range(_CHUNK_ROWS // _WRITE_ROWS):
                r = row_slice(chunk, part, _WRITE_ROWS)
                pltpu.make_async_copy(
                    buf.at[:, r], o_hbm.at[:, r], write_sem
                ).start()

        def compute(chunk):
            r = row_slice(chunk, 0, _CHUNK_ROWS)
            pixels = buf[:, r, :].reshape(_GROUPS * _CHUNK_ROWS, C)
            depthwise = pixels * dw_vmem[0]
            out = jnp.dot(
                depthwise, pw_vmem[...], preferred_element_type=jnp.float32)
            buf[:, r, :] = out.astype(buf.dtype).reshape(
                _GROUPS, _CHUNK_ROWS, C)

        pw_copy = pltpu.make_async_copy(pw_hbm, pw_vmem, weight_sems.at[0])
        dw_copy = pltpu.make_async_copy(dw_hbm, dw_vmem, weight_sems.at[1])
        pw_copy.start()
        dw_copy.start(priority=1)
        lax.fori_loop(0, _PREFETCH, lambda c, _: start_read(c), None)
        pw_copy.wait()
        dw_copy.wait()

        def read_phase(step, _):
            for batch in range(n_batches):
                if edges[batch] < read_steps:
                    pl.when(step == edges[batch])(
                        functools.partial(wait_batch, batch))
            compute(step)
            start_read(_PREFETCH + 2 * step)
            start_read(_PREFETCH + 2 * step + 1)

        lax.fori_loop(0, read_steps, read_phase, None)
        for batch in range(n_batches - 1):
            if edges[batch] >= read_steps:
                wait_batch(batch)

        def write_phase(step, _):
            started = jnp.minimum(2 * (step - read_steps), step - 1)
            front = jnp.minimum(2 * (step - read_steps + 1), step)
            pl.when(front - started == 2)(lambda: start_write(front - 2))
            start_write(front - 1)
            pl.when(step == n_chunks - 1)(
                functools.partial(wait_batch, n_batches - 1))
            compute(step)

        lax.fori_loop(read_steps, n_chunks, write_phase, None)
        start_write(n_chunks - 1)
        pltpu.make_async_copy(buf, o_hbm, write_sem).wait()

    hbm = pl.BlockSpec(memory_space=pltpu.HBM)
    out = pl.pallas_call(
        kernel,
        in_specs=[hbm, hbm, hbm],
        out_specs=hbm,
        out_shape=jax.ShapeDtypeStruct((_GROUPS, rows, C), x.dtype),
        scratch_shapes=[
            pltpu.VMEM((_GROUPS, rows, C), x.dtype),
            pltpu.VMEM(dw.shape, dw.dtype),
            pltpu.VMEM(pw.shape, pw.dtype),
            pltpu.SemaphoreType.DMA((n_batches,)),
            pltpu.SemaphoreType.DMA,
            pltpu.SemaphoreType.DMA((2,)),
        ],
        compiler_params=pltpu.CompilerParams(vmem_limit_bytes=120 << 20),
    )(x.reshape(_GROUPS, rows, C), dw, pw)
    return out.reshape(B, H, W, C)
```
